```python
import jax
import jax.numpy as jnp

def _softmax(x, axis=-1):
    return jax.nn.softmax(x, axis=axis)

def _gelu(x):
    return jax.nn.gelu(x, approximate=True)

def _silu(x):
    return jax.nn.silu(x)

def _sigmoid(x):
    return jax.nn.sigmoid(x)

def _layernorm(x, axis=-1, eps=1e-05):
    m = jnp.mean(x, axis=axis, keepdims=True)
    v = jnp.var(x, axis=axis, keepdims=True)
    return (x - m) / jnp.sqrt(v + eps)

def _scatter_add(tgt, idx, src, axis=0):
    return tgt.at[idx].add(src)

def _segment_sum(src, seg, n):
    return jax.ops.segment_sum(src, seg, n)

class _Rng:

    def __init__(self, key):
        self._k = key

    def _next(self):
        self._k, sub = jax.random.split(self._k)
        return sub

    def normal(self, shape):
        return jax.random.normal(self._next(), shape, dtype=jnp.bfloat16)

    def randint(self, lo, hi, shape):
        return jax.random.randint(self._next(), shape, lo, hi, dtype=jnp.int32)

    def uniform(self, shape, lo=0.0, hi=1.0):
        return jax.random.uniform(self._next(), shape, jnp.bfloat16, lo, hi)

    def permutation(self, n):
        return jax.random.permutation(self._next(), n)
kernel_name = 'standalone__conformer_conv_module__speech'

def setup_inputs():
    _rng = _Rng(jax.random.key(int.from_bytes(__import__("os").urandom(4), "little")))
    _w = lambda a: (lambda t: t.astype(jnp.bfloat16) if jnp.issubdtype(t.dtype, jnp.floating) else t)(jnp.asarray(a))
    B, T, D, K = (2, 16000, 256, 31)
    return {'x': _w((lambda *s: _rng.normal(s) * 0.05)(B, T, D)), 'w_pw1': _w((lambda *s: _rng.normal(s) * 0.05)(D, 2 * D)), 'dw': _w((lambda *s: _rng.normal(s) * 0.05)(K, D)), 'w_pw2': _w((lambda *s: _rng.normal(s) * 0.05)(D, D))}

def reference(x, w_pw1, dw, w_pw2):
    B, T, D = x.shape
    K = dw.shape[0]
    h = x @ w_pw1
    a, b = (h[..., :D].copy(), h[..., D:].copy())
    h = a * _sigmoid(b)
    pad = K // 2
    hp = jnp.pad(h, ((0, 0), (pad, pad), (0, 0)))
    out = jnp.zeros_like(h)
    for i in range(K):
        out = out + hp[:, i:i + T, :] * dw[i][None, None, :]
    return _silu(out) @ w_pw2
```

```python
import functools

import jax
import jax.numpy as jnp
from jax import lax
import jax.experimental.pallas as pl
import jax.experimental.pallas.tpu as pltpu

L = 128
OFF = 64
NT = (((1,), (1,)), ((), ()))
bf16, f32, u32, i32 = jnp.bfloat16, jnp.float32, jnp.uint32, jnp.int32


def _kernel(x_hbm, w1_ref, dw_ref, w2_ref, o_hbm,
            xbuf, g_ref, s_ref, w1t_ref, w2p_ref, dwp_ref, dwt_ref, isem, osem,
            *, T, D, K, CP, SP, N1, DB, U2, N3, OB, LA, XT, U3, phases):
    NO = T // L
    NI = NO + 1
    M = 128
    nin = len(DB)
    eb = [sum(DB[:d]) for d in range(nin + 1)]
    assert eb[-1] == NI

    def in_copy(b, d):
        lo = max(eb[d] * L - OFF, 0)
        hi = min(eb[d + 1] * L - OFF, T)
        return pltpu.make_async_copy(
            x_hbm.at[b, pl.ds(lo, hi - lo)],
            xbuf.at[b, pl.ds(lo + OFF, hi - lo)], isem.at[b, d])

    for d in range(LA):
        for b in range(2):
            in_copy(b, d).start()

    for b in range(2):
        xbuf[b, pl.ds(0, OFF), :] = jnp.zeros((OFF, D), bf16)
        xbuf[b, pl.ds(T + OFF, L - OFF), :] = jnp.zeros((L - OFF, D), bf16)
    w1t_ref[...] = pltpu.bitcast((w1_ref[...].astype(f32) * 0.5).T.astype(bf16), u32)
    w2u = pltpu.bitcast(w2_ref[...], u32)
    w2p_ref[...] = jnp.concatenate(
        [pltpu.bitcast(w2u << 16, f32), pltpu.bitcast(w2u & u32(0xFFFF0000), f32)],
        axis=0).astype(bf16)
    dwp_ref[...] = jnp.zeros(dwp_ref.shape, f32)
    dwp_ref[pl.ds(0, K), :] = dw_ref[...].astype(f32) * 0.5
    dwt_ref[...] = dwp_ref[...].T
    for j in range(NI, M + 1):
        g_ref[pl.ds(j * CP, D), :] = jnp.zeros((D, L), u32)

    def p1(j0, N1, i, _):
        j = j0 + i * N1
        t0 = pl.multiple_of(j * L, L)
        gs = []
        for b in range(2):
            h = lax.dot_general(pltpu.bitcast(w1t_ref[...], bf16), xbuf[b, pl.ds(t0, N1 * L), :], NT,
                                preferred_element_type=f32)
            a = h[:D]
            gs.append(a + a * jnp.tanh(h[D:]))
        g = pltpu.pack_elementwise(gs, packed_dtype=bf16)
        for n in range(N1):
            g_ref[pl.ds((j + n) * CP, D), :] = g[:, n * L:(n + 1) * L]

    for d in range(nin):
        for b in range(2):
            in_copy(b, d).wait()
            if d + LA < nin:
                in_copy(b, d + LA).start()
        if 1 in phases:
            n1 = min(N1, DB[d])
            lax.fori_loop(0, DB[d] // n1, functools.partial(p1, eb[d], n1), None)

    sh = OFF - K // 2
    row = lax.broadcasted_iota(i32, (L, L), 0)
    col = lax.broadcasted_iota(i32, (L, L), 1)
    cur = (col - row - sh) >= 0
    ones = jnp.ones((L, L), f32)
    mcur = pltpu.bitcast(jnp.where(cur, ones, 0.0).astype(bf16), u32)
    mcur = (mcur >> 7 & u32(0x00010001)) * u32(0xFFFF)

    def conv(c):
        r = jnp.broadcast_to(dwt_ref[pl.ds(c, 1), :], (16, L))
        p = pltpu.roll(r, sh, 1, stride=1, stride_axis=0).astype(bf16)
        p = pltpu.bitcast(p, u32)
        circ = jnp.concatenate(
            [p] + [pltpu.roll(p, 16 * m, 1) for m in range(1, L // 16)], axis=0)
        top = circ & mcur
        w = jnp.concatenate([top, circ ^ top], axis=1)
        l0 = g_ref[pl.ds(c, M, stride=CP), :]
        l1 = g_ref[pl.ds(c + CP, M, stride=CP), :]
        lhs = pltpu.bitcast(jnp.concatenate([l0, l1], axis=1), bf16)
        y = lax.dot_general(lhs, pltpu.bitcast(w, bf16), NT,
                            preferred_element_type=f32)
        return y + y * jnp.tanh(y)

    def p2(i, _):
        for u in range(U2):
            cp = i * U2 + u
            s = pltpu.pack_elementwise([conv(2 * cp), conv(2 * cp + 1)],
                                       packed_dtype=bf16)
            s_ref[pl.ds(cp * SP, 2 * M), :] = s

    if 2 in phases:
        lax.fori_loop(0, D // 2 // U2, p2, None)

    def out_copy(b, d):
        sl = pl.ds(d * OB * L, OB * L)
        return pltpu.make_async_copy(xbuf.at[b, sl], o_hbm.at[b, sl], osem.at[b, d])

    def p3(b, i, _):
        ss = []
        for n in range(N3):
            s = s_ref[pl.ds(2 * (i * N3 + n) + b, D // 2, stride=SP), :]
            if not XT:
                ss.append(pltpu.bitcast(s, bf16).T)
                continue
            s = s.T
            ss.append(jnp.concatenate(
                [pltpu.bitcast(s << 16, f32), pltpu.bitcast(s & u32(0xFFFF0000), f32)],
                axis=1).astype(bf16))
        o = jnp.dot(jnp.concatenate(ss, axis=0), w2p_ref[...] if XT else w2_ref[...],
                    preferred_element_type=f32)
        t0 = pl.multiple_of(i * (N3 * L), N3 * L)
        xbuf[b, pl.ds(t0, N3 * L), :] = o.astype(bf16)

    nout = NO // OB

    def p3o(b, q, _):
        for u in range(U3):
            d = q * U3 + u
            for v in range(OB // N3):
                if 3 in phases:
                    p3(b, d * (OB // N3) + v, None)
            out_copy(b, d).start()

    for b in range(2):
        lax.fori_loop(0, nout // U3, functools.partial(p3o, b), None)
    for b in range(2):
        lax.fori_loop(0, nout, lambda d, _, b=b: out_copy(b, d).wait(), None)


def _call(x, w_pw1, dw, w_pw2, CP=257, SP=257, N1=12, DB=(2,4,12,24,36,48), U2=64, N3=5, OB=5, LA=2, U3=5, XT=1,
          phases=(1, 2, 3)):
    B, T, D = x.shape
    K = dw.shape[0]
    assert B == 2 and T % L == 0 and T // L < 128 and K // 2 <= OFF
    NO = T // L
    vm = pl.BlockSpec(memory_space=pltpu.VMEM)
    return pl.pallas_call(
        functools.partial(_kernel, T=T, D=D, K=K, CP=CP, SP=SP, N1=N1, DB=DB,
                          U2=U2, N3=N3, OB=OB, LA=LA, U3=U3, XT=XT, phases=phases),
        in_specs=[pl.BlockSpec(memory_space=pl.ANY), vm, vm, vm],
        out_specs=pl.BlockSpec(memory_space=pl.ANY),
        out_shape=jax.ShapeDtypeStruct((B, T, D), bf16),
        scratch_shapes=[
            pltpu.VMEM((B, T + L, D), bf16),
            pltpu.VMEM((-(-129 * CP // 8) * 8, L), u32),
            pltpu.VMEM((D // 2 * SP, L), u32),
            pltpu.VMEM((D, D), u32),
            pltpu.VMEM((D, D), bf16),
            pltpu.VMEM((L, D), f32),
            pltpu.VMEM((D, L), f32),
            pltpu.SemaphoreType.DMA((B, len(DB))),
            pltpu.SemaphoreType.DMA((B, NO // OB)),
        ],
        compiler_params=pltpu.CompilerParams(vmem_limit_bytes=100 * 2**20),
    )(x, w_pw1, dw, w_pw2)


@jax.jit
def pallas_standalone__conformer_conv_module__speech_kernel(x, w_pw1, dw, w_pw2):
    return _call(x, w_pw1, dw, w_pw2)
```
